```python
import os as _os
_os.environ.setdefault("JAX_PLATFORMS", "cpu")
import jax
import jax.numpy as jnp

def _softmax(x, axis=-1):
    return jax.nn.softmax(x, axis=axis)
def _gelu(x):
    return jax.nn.gelu(x, approximate=True)
def _silu(x):
    return jax.nn.silu(x)
def _sigmoid(x):
    return jax.nn.sigmoid(x)
def _layernorm(x, axis=-1, eps=1e-5):
    m = jnp.mean(x, axis=axis, keepdims=True)
    v = jnp.var(x, axis=axis, keepdims=True)
    return (x - m) / jnp.sqrt(v + eps)
def _scatter_add(tgt, idx, src, axis=0):
    return tgt.at[idx].add(src)
def _segment_sum(src, seg, n):
    return jax.ops.segment_sum(src, seg, n)
class _Rng:
    def __init__(self, key):
        self._k = key
    def _next(self):
        self._k, sub = jax.random.split(self._k)
        return sub
    def normal(self, shape):
        return jax.random.normal(self._next(), shape, dtype=jnp.bfloat16)
    def randint(self, lo, hi, shape):
        return jax.random.randint(self._next(), shape, lo, hi, dtype=jnp.int32)
    def uniform(self, shape, lo=0.0, hi=1.0):
        return jax.random.uniform(self._next(), shape, jnp.bfloat16, lo, hi)
    def permutation(self, n):
        return jax.random.permutation(self._next(), n)


kernel_name = 'gated_mix__linear_attn_block__mixer_token_mlp__prompt'

def setup_inputs():
    _rng = _Rng(jax.random.key(int.from_bytes(__import__("os").urandom(4), "little")))
    _w = (lambda a: (lambda t: t.astype(jnp.bfloat16) if jnp.issubdtype(t.dtype, jnp.floating) else t)(jnp.asarray(a)))
    def _A_setup():
        B, S, D = 1, 2048, 512
        return {
            "x": _w((lambda *s: _rng.normal(s) * 0.05)(B, S, D)),
            "wqkv": _w((lambda *s: _rng.normal(s) * 0.8)(D, 3 * D)),
            "wo": _w((lambda *s: _rng.normal(s) * 0.05)(D, D)),
        }
    _A_in = _A_setup()

    def _B_setup():
        B, S, D, F = 1, 2048, 512, 1792
        return {
            "x": _w((lambda *s: _rng.normal(s) * 0.05)(B, S, D)),
            "w1": _w((lambda *s: _rng.normal(s) * 0.1)(S, F) * (S ** -0.5)),
            "b1": _w((lambda *s: _rng.normal(s) * 0.1)(F) * 0.02),
            "w2": _w((lambda *s: _rng.normal(s) * 0.1)(F, S) * (F ** -0.5)),
            "b2": _w((lambda *s: _rng.normal(s) * 0.1)(S) * 0.02),
        }
    _B_in = _B_setup()

    return {
        "A_x": _A_in["x"],
        "A_wqkv": _A_in["wqkv"],
        "A_wo": _A_in["wo"],
        "B_x": _B_in["x"],
        "B_w1": _B_in["w1"],
        "B_b1": _B_in["b1"],
        "B_w2": _B_in["w2"],
        "B_b2": _B_in["b2"],
        "gate_w": _w((lambda *s: _rng.normal(s) * 0.05)(512) * 16.0),
    }

def reference(A_x, A_wqkv, A_wo, B_x, B_w1, B_b1, B_w2, B_b2, gate_w):
    def _A_ref(x, wqkv, wo):
        B, S, D = x.shape
        H = 32; Dh = D // H
        qkv = (lambda x, *d: x.transpose(*d))((x @ wqkv).reshape(B, S, 3, H, Dh), 2, 0, 3, 1, 4)
        q, k, v = qkv[0], qkv[1], qkv[2]
        phi = lambda t: jnp.where(t > 0, t + 1, jnp.exp(t)) + 1e-6
        pq, pk = phi(q), phi(k)
        kv = jnp.einsum("bhsd,bhse->bhde", pk, v)
        z = jnp.einsum("bhsd->bhd", pk)
        num = jnp.einsum("bhqd,bhde->bhqe", pq, kv)
        den = jnp.einsum("bhqd,bhd->bhq", pq, z)[..., None] + 1e-6
        o = num / den
        return (lambda x, *d: x.transpose(*d))(o, 0, 2, 1, 3).reshape(B, S, D) @ wo

    def _B_ref(x, w1, b1, w2, b2):
        B, S, D = x.shape
        h = _layernorm(x, axis=-1)
        u = jnp.einsum("bsd,sf->bdf", h, w1) + b1
        u = _gelu(u)
        y = jnp.einsum("bdf,fs->bds", u, w2) + b2
        return (lambda x, *d: x.transpose(*d))(y, 0, 2, 1)

    x = A_x
    g = _sigmoid((x * gate_w).sum(-1, keepdims=True))
    a = _A_ref(x, A_wqkv, A_wo)
    b = _B_ref(x, B_w1, B_b1, B_w2, B_b2)
    return g * a + (1 - g) * b
```

```python
import jax
import jax.numpy as jnp
from jax import lax
from jax.experimental import pallas as pl
from jax.experimental.pallas import tpu as pltpu

S, D, F, H, DH = 2048, 512, 1792, 32, 16
BF, F32, U32 = jnp.bfloat16, jnp.float32, jnp.uint32
PAD = 16

_X0, _X1, _X2, _X3 = ("x", 0, 256), ("x", 256, 256), ("x", 512, 512), ("x", 1024, 1024)
_WK = [("wk", 128 * i, 128) for i in range(4)]
_WQ, _WV, _WO = ("wq", 0, D), ("wv", 0, D), ("wo",)
_GW, _B1, _B2, _W1 = ("gw",), ("b1",), ("b2",), ("w1",)
_YCHUNKS = [(0, 1536), (1536, 256), (1792, 128), (1920, 128)]
_W2 = [("w2", a, n) for a, n in _YCHUNKS]
_OUT = [("o", 0, 768), ("o", 768, 768), ("o", 1536, 256), ("o", 1792, 128), ("o", 1920, 128)]
_INPUTS = [_X0, _WK[0], _WK[1], _X1, _WK[2], _WK[3], _X2, _WQ, _GW, _X3, _B1, _W1, _WV, _WO, _B2] + _W2
_COPIES = _INPUTS + _OUT


def _dot(a, b):
    return jnp.dot(a, b, preferred_element_type=F32)


def _phi(t):
    return jnp.where(t > 0, t + 1.0, jnp.exp(t)) + 1e-6


class _Packed:
    def __init__(self, ref):
        self.ref = ref

    @staticmethod
    def _idx(idx):
        r, c = idx
        r = slice(None) if isinstance(r, slice) else pl.ds(r.start // 2, r.size // 2)
        return r, c

    def __getitem__(self, idx):
        r, c = self._idx(idx)
        return pltpu.bitcast(self.ref[r, c], BF)

    def __setitem__(self, idx, val):
        r, c = self._idx(idx)
        self.ref[r, c] = pltpu.bitcast(val, U32)


def _kernel(x_hbm, wqkv_hbm, wo_hbm, w1_hbm, b1_hbm, w2_hbm, b2_hbm, gw_hbm, out_hbm,
            x_v, wq_v, wk_v, wv_v, wo_v, w1_v, b1_v, b2_v, gw_v,
            wqT_v, wvT_v, woT_v, xT_v, hT_v, pqT_v, pk_v, PT_v, KV_v, MT_v, g_v,
            gate_v, mean_v, z_v, zc0_v, zc_v, R_v, out_v, sems, *w2_vs):
    wqT_v, wvT_v, woT_v, xT_v, hT_v, pqT_v, pk_v, PT_v, KV_v, MT_v, g_v = [_Packed(wqT_v), _Packed(wvT_v), _Packed(woT_v), _Packed(xT_v), _Packed(hT_v), pqT_v, _Packed(pk_v), _Packed(PT_v), KV_v, _Packed(MT_v), _Packed(g_v)]
    w2_v = dict(zip(_W2, w2_vs))
    every = slice(None)

    def copy(name):
        kind, sem = name[0], sems.at[_COPIES.index(name)]
        if kind == "x":
            rows = pl.ds(name[1], name[2])
            return pltpu.make_async_copy(x_hbm.at[0, rows, :], x_v.at[rows, :], sem)
        if kind == "o":
            rows = pl.ds(name[1], name[2])
            return pltpu.make_async_copy(out_v.at[rows, :], out_hbm.at[0, rows, :], sem)
        if kind in ("wq", "wk", "wv"):
            off, dst = {"wq": (0, wq_v), "wk": (D, wk_v), "wv": (2 * D, wv_v)}[kind]
            return pltpu.make_async_copy(wqkv_hbm.at[:, pl.ds(off + name[1], name[2])],
                                         dst.at[pl.ds(0, D), pl.ds(name[1], name[2])], sem)
        if kind == "w2":
            return pltpu.make_async_copy(w2_hbm.at[:, pl.ds(name[1], name[2])], w2_v[name].at[pl.ds(0, F), :], sem)
        src, dst = {"wo": (wo_hbm, wo_v), "w1": (w1_hbm, w1_v.at[pl.ds(0, S), :]),
                    "b1": (b1_hbm, b1_v), "b2": (b2_hbm, b2_v), "gw": (gw_hbm, gw_v)}[kind]
        return pltpu.make_async_copy(src, dst, sem)

    def start(*names):
        for name in names:
            copy(name).start()

    def wait(*names):
        for name in names:
            copy(name).wait()

    def anchor(dst, row, src, r0, c0, col=0):
        dst[pl.ds(row, PAD), pl.ds(col, 128)] = src[pl.ds(r0, PAD), pl.ds(c0, 128)]

    z_seen = set()

    def k_proj(a, n, c0=0, cn=D):
        rows, cols = pl.ds(a, n), pl.ds(c0, cn)
        pk = _phi(_dot(x_v[rows, :], wk_v[0:D, cols]))
        pk_v[rows, cols] = pk.astype(BF)
        part = jnp.sum(pk.reshape(n // 8, 8, cn), axis=0)
        for j in range(c0 // 128, (c0 + cn) // 128):
            js, ps = slice(j * 128, (j + 1) * 128), slice(j * 128 - c0, (j + 1) * 128 - c0)
            if j in z_seen:
                z_v[:, js] += part[:, ps]
            else:
                z_v[:, js] = part[:, ps]
                z_seen.add(j)

    def transpose_x(a, n):
        xT_v[every, pl.ds(a, n)] = x_v[pl.ds(a, n), :].T

    def q_proj(a, n):
        cols = pl.ds(a, n)
        r = _dot(wqT_v[every, every], xT_v[every, cols])
        pqT_v[every, cols] = _phi(r[:D]).astype(BF)
        gate_v[:, cols] = jnp.broadcast_to(1.0 / (1.0 + jnp.exp(-r[D:D + 1])), (8, n))
        mean_v[:, cols] = jnp.broadcast_to(r[D + 1:D + 2], (8, n))

    def layernorm(a, n):
        for t in range(a, a + n, 128):
            cols = pl.ds(t, 128)
            xm = xT_v[every, cols].astype(F32) - mean_v[0:1, cols]
            var = jnp.sum(xm * xm, axis=0, keepdims=True) * (1.0 / D)
            mean_v[4:5, cols] = var
            hT_v[every, cols] = (xm * lax.rsqrt(var + 1e-5)).astype(BF)

    def p_proj(a, n):
        PT_v[every, pl.ds(a, n)] = _dot(xT_v[every, every], pk_v[every, pl.ds(a, n)]).astype(BF)

    def kv_block(j):
        row_head = lax.broadcasted_iota(jnp.int32, (128, 128), 0) // DH
        col_head = lax.broadcasted_iota(jnp.int32, (128, 128), 1) // DH
        js = pl.ds(j * 128, 128)
        kvT = _dot(wvT_v[js, every], PT_v[every, js])
        KV_v[js, every] = jnp.where(row_head == col_head, kvT, 0.0).astype(BF)

    def m_block(j):
        js = pl.ds(j * 128, 128)
        MT_v[every, js] = _dot(woT_v[every, js], KV_v[js, every]).astype(BF)

    def mixer_up(a, n):
        b1 = b1_v[...].astype(F32).reshape(1, F)
        u = _dot(hT_v[every, every], w1_v[0:S, pl.ds(a, n)]) + b1[:, a:a + n]
        g_v[every, pl.ds(a, n)] = jax.nn.gelu(u, approximate=True).astype(BF)

    def normalized_q(a, n):
        sub = lax.broadcasted_iota(jnp.int32, (8, 128), 0)
        m4, m2, m1 = sub < 4, (sub & 2) == 0, (sub & 1) == 0
        outs = []
        for t in range(a, a + n, 128):
            p = pqT_v[every, pl.ds(t, 128)].astype(F32)
            pz = p * zc_v[...]
            rows = []
            for grp in range(H // 8):
                h0 = grp * 8 * DH
                A = [pz[h0 + i * DH:h0 + i * DH + 8] + pz[h0 + i * DH + 8:h0 + (i + 1) * DH] for i in range(8)]
                B = [jnp.where(m4, A[i], A[i + 1]) + pltpu.roll(jnp.where(m4, A[i + 1], A[i]), 4, 0)
                     for i in range(0, 8, 2)]
                C = [jnp.where(m2, B[i] + pltpu.roll(B[i], 6, 0), B[i + 1] + pltpu.roll(B[i + 1], 2, 0))
                     for i in range(0, 4, 2)]
                den = jnp.where(m1, C[0] + pltpu.roll(C[0], 7, 0), C[1] + pltpu.roll(C[1], 1, 0)) + 1e-6
                inv = 1.0 / den
                for i in range(8):
                    s = ((i & 1) << 2) | (i & 2) | ((i >> 2) & 1)
                    rows.append(jnp.broadcast_to(inv[s:s + 1, :], (DH, 128)))
            outs.append((p * jnp.concatenate(rows, axis=0)).astype(BF))
        return jnp.concatenate(outs, axis=1) if len(outs) > 1 else outs[0]

    def mixer_down(chunk):
        a, n = chunk
        cols = pl.ds(a, n)
        b2 = b2_v[...].astype(F32).reshape(1, S)
        y = _dot(g_v[every, every], w2_v[("w2", a, n)][0:F, :])
        R_v[:, cols] = (1.0 - gate_v[0:1, cols]) * (y + b2[:, a:a + n])

    def attn_out(a, n):
        cols = pl.ds(a, n)
        R_v[:, cols] = R_v[:, cols] + gate_v[0:1, cols] * _dot(MT_v[every, every], normalized_q(a, n))

    def emit(a, n):
        out_v[pl.ds(a, n), :] = R_v[:, pl.ds(a, n)].T.astype(BF)

    start(*_INPUTS)

    wait(_X0, _WK[0])
    k_proj(0, 256, 0, 128)
    transpose_x(0, 256)
    wait(_WK[1])
    k_proj(0, 256, 128, 128)
    wait(_X1)
    k_proj(256, 256, 0, 256)
    transpose_x(256, 256)
    wait(_WK[2])
    k_proj(0, 512, 256, 128)
    wait(_WK[3])
    k_proj(0, 512, 384, 128)
    wait(_X2)
    k_proj(512, 256)
    transpose_x(512, 256)
    k_proj(768, 256)
    transpose_x(768, 256)

    anchor(wq_v, D, pk_v, 768, 0)
    wait(_WQ, _GW)
    wqT_v[pl.ds(0, D), every] = wq_v[0:D, :].T
    aug_row = lax.broadcasted_iota(jnp.int32, (16, D), 0)
    gw = jnp.broadcast_to(gw_v[...].astype(F32).reshape(1, D), (16, D))
    wqT_v[pl.ds(D, 16), every] = jnp.where(aug_row == 0, gw, jnp.where(aug_row == 1, 1.0 / D, 0.0)).astype(BF)
    q_proj(0, 512)

    wait(_X3)
    k_proj(1024, 1024)
    transpose_x(1024, 1024)
    q_proj(512, 512)
    q_proj(1024, 1024)
    for c in range(0, S, 512):
        layernorm(c, 512)
    z_row = jnp.sum(z_v[...], axis=0, keepdims=True)
    zc0_v[...] = jnp.broadcast_to(z_row, (128, D)).T
    for j in range(4):
        p_proj(j * 128, 128)

    for t in range(4):
        anchor(w1_v, S, hT_v, D - PAD, 1536 + 128 * t, col=128 * (t + 1))
    anchor(w1_v, S, PT_v, 0, 384)
    wait(_W1, _B1, _WV, _WO)
    wvT_v[every, every] = wv_v[0:D, :].T
    woT_v[every, every] = wo_v[0:D, :].T

    mixer_up(0, 256)
    for j in range(4):
        kv_block(j)
    mixer_up(256, 256)
    for j in range(4):
        m_block(j)
    for f in range(2, 5):
        mixer_up(f * 256, 256)
    anchor(w2_v[_W2[0]], F, g_v, 0, 1024)
    wait(_W2[0], _B2)
    mixer_up(1280, 256)
    tie = g_v[pl.ds(0, 16), pl.ds(1408, 128)].astype(F32)[0:8] * 0.0
    zc_v[...] = zc0_v[...] + jnp.concatenate([tie] * (D // 8), axis=0)
    mixer_up(1536, 256)

    mixer_down(_YCHUNKS[0])
    for a in range(0, 1536, 256):
        attn_out(a, 256)
    wait(_W2[1])
    mixer_down(_YCHUNKS[1])
    attn_out(1536, 256)
    emit(0, 1536)
    start(_OUT[0], _OUT[1])
    wait(_W2[2])
    mixer_down(_YCHUNKS[2])
    attn_out(1792, 128)
    emit(1536, 256)
    start(_OUT[2])
    wait(_W2[3])
    mixer_down(_YCHUNKS[3])
    attn_out(1920, 128)
    emit(1792, 128)
    start(_OUT[3])
    wait(_OUT[0])
    emit(1920, 128)
    start(_OUT[4])
    wait(_OUT[1])
    wait(_OUT[2], _OUT[3], _OUT[4])


@jax.jit
def pallas_gated_mix__linear_attn_block__mixer_token_mlp__prompt_kernel(
    A_x: jax.Array,
    A_wqkv: jax.Array,
    A_wo: jax.Array,
    B_x: jax.Array,
    B_w1: jax.Array,
    B_b1: jax.Array,
    B_w2: jax.Array,
    B_b2: jax.Array,
    gate_w: jax.Array,
):
    del B_x
    hbm = pl.BlockSpec(memory_space=pl.ANY)
    V = pltpu.VMEM
    scratch = [
        V((S, D), BF), V((D + PAD, D), BF), V((D, D), BF), V((D, D), BF), V((D, D), BF),
        V((S + PAD, F), BF), V((F,), BF), V((S,), BF), V((D,), BF),
        V(((D + 16) // 2, D), U32), V(((D) // 2, D), U32), V(((D) // 2, D), U32), V(((D) // 2, S), U32), V(((D) // 2, S), U32), V((D, S), BF), V(((S) // 2, D), U32), V(((D) // 2, D), U32), V((D, 128), BF), V(((D) // 2, D), U32), V(((D) // 2, F), U32),
        V((8, S), F32), V((8, S), F32), V((8, D), F32), V((D, 128), F32), V((D, 128), F32), V((D, S), F32), V((S, D), BF),
        pltpu.SemaphoreType.DMA((len(_COPIES),)),
    ] + [V((F + PAD, n), BF) for _, n in _YCHUNKS]
    return pl.pallas_call(
        _kernel,
        out_shape=jax.ShapeDtypeStruct((1, S, D), BF),
        in_specs=[hbm] * 8,
        out_specs=hbm,
        scratch_shapes=scratch,
        compiler_params=pltpu.CompilerParams(
            vmem_limit_bytes=100 * 1024 * 1024,
            flags={"XLA_TPU_RESCHEDULE_DMA_DONES": True},
            disable_semaphore_checks=True,
            disable_bounds_checks=True,
        ),
    )(A_x, A_wqkv, A_wo, B_w1, B_b1, B_w2, B_b2, gate_w)
```

```python
import jax
import jax.numpy as jnp
from jax import lax
from jax.experimental import pallas as pl
from jax.experimental.pallas import tpu as pltpu

S, D, F, H, DH = 2048, 512, 1792, 32, 16
BF, F32, U32 = jnp.bfloat16, jnp.float32, jnp.uint32
PAD = 16

_X0, _X1, _X2, _X3 = ("x", 0, 256), ("x", 256, 256), ("x", 512, 512), ("x", 1024, 1024)
_WK = [("wk", 128 * i, 128) for i in range(4)]
_WQ, _WV, _WO = ("wq", 0, D), ("wv", 0, D), ("wo",)
_GW, _B1, _B2, _W1 = ("gw",), ("b1",), ("b2",), ("w1",)
_LATE = ("late",)
_YCHUNKS = [(0, 1536), (1536, 256), (1792, 128), (1920, 128)]
_W2 = [("w2", a, n) for a, n in _YCHUNKS]
_OUT = [("o", 0, 768), ("o", 768, 768), ("o", 1536, 256), ("o", 1792, 128), ("o", 1920, 128)]
_INPUTS = [_X0, _WK[0], _WK[1], _X1, _WK[2], _WK[3], _X2, _WQ, _GW, _X3, _B1, _W1, _WV, _WO, _B2] + _W2 + [_LATE]
_COPIES = _INPUTS + _OUT


def _dot(a, b):
    return jnp.dot(a, b, preferred_element_type=F32)


def _phi(t):
    return jnp.where(t > 0, t + 1.0, jnp.exp(t)) + 1e-6


class _Packed:
    def __init__(self, ref):
        self.ref = ref

    @staticmethod
    def _idx(idx):
        r, c = idx
        r = slice(None) if isinstance(r, slice) else pl.ds(r.start // 2, r.size // 2)
        return r, c

    def __getitem__(self, idx):
        r, c = self._idx(idx)
        return pltpu.bitcast(self.ref[r, c], BF)

    def __setitem__(self, idx, val):
        r, c = self._idx(idx)
        self.ref[r, c] = pltpu.bitcast(val, U32)


def _kernel(x_hbm, wqkv_hbm, wo_hbm, w1_hbm, b1_hbm, w2_hbm, b2_hbm, gw_hbm, out_hbm,
            x_v, wq_v, wk_v, wv_v, wo_v, w1_v, b1_v, b2_v, gw_v,
            wqT_v, wvT_v, woT_v, xT_v, hT_v, pqT_v, pk_v, PT_v, KV_v, MT_v, g_v,
            gate_v, mean_v, z_v, zc0_v, zc_v, zc2_v, late_v, R_v, out_v, sems, *w2_vs):
    wqT_v, wvT_v, woT_v, xT_v, hT_v, pqT_v, pk_v, PT_v, KV_v, MT_v, g_v = [_Packed(wqT_v), _Packed(wvT_v), _Packed(woT_v), _Packed(xT_v), _Packed(hT_v), pqT_v, _Packed(pk_v), _Packed(PT_v), KV_v, _Packed(MT_v), _Packed(g_v)]
    w2_v = dict(zip(_W2, w2_vs))
    every = slice(None)

    def copy(name):
        kind, sem = name[0], sems.at[_COPIES.index(name)]
        if kind == "x":
            rows = pl.ds(name[1], name[2])
            return pltpu.make_async_copy(x_hbm.at[0, rows, :], x_v.at[rows, :], sem)
        if kind == "o":
            rows = pl.ds(name[1], name[2])
            return pltpu.make_async_copy(out_v.at[rows, :], out_hbm.at[0, rows, :], sem)
        if kind in ("wq", "wk", "wv"):
            off, dst = {"wq": (0, wq_v), "wk": (D, wk_v), "wv": (2 * D, wv_v)}[kind]
            return pltpu.make_async_copy(wqkv_hbm.at[:, pl.ds(off + name[1], name[2])],
                                         dst.at[pl.ds(0, D), pl.ds(name[1], name[2])], sem)
        if kind == "w2":
            return pltpu.make_async_copy(w2_hbm.at[:, pl.ds(name[1], name[2])], w2_v[name].at[pl.ds(0, F), :], sem)
        src, dst = {"wo": (wo_hbm, wo_v), "w1": (w1_hbm, w1_v.at[pl.ds(0, S), :]),
                    "b1": (b1_hbm, b1_v), "b2": (b2_hbm, b2_v), "gw": (gw_hbm, gw_v), "late": (b2_hbm, late_v)}[kind]
        return pltpu.make_async_copy(src, dst, sem)

    def start(*names):
        for name in names:
            copy(name).start()

    def wait(*names):
        for name in names:
            copy(name).wait()

    def anchor(dst, row, src, r0, c0, col=0):
        dst[pl.ds(row, PAD), pl.ds(col, 128)] = src[pl.ds(r0, PAD), pl.ds(c0, 128)]

    z_seen = set()

    def k_proj(a, n, c0=0, cn=D):
        rows, cols = pl.ds(a, n), pl.ds(c0, cn)
        pk = _phi(_dot(x_v[rows, :], wk_v[0:D, cols]))
        pk_v[rows, cols] = pk.astype(BF)
        part = jnp.sum(pk.reshape(n // 8, 8, cn), axis=0)
        for j in range(c0 // 128, (c0 + cn) // 128):
            js, ps = slice(j * 128, (j + 1) * 128), slice(j * 128 - c0, (j + 1) * 128 - c0)
            if j in z_seen:
                z_v[:, js] += part[:, ps]
            else:
                z_v[:, js] = part[:, ps]
                z_seen.add(j)

    def transpose_x(a, n):
        xT_v[every, pl.ds(a, n)] = x_v[pl.ds(a, n), :].T

    def q_proj(a, n):
        cols = pl.ds(a, n)
        r = _dot(wqT_v[every, every], xT_v[every, cols])
        pqT_v[every, cols] = _phi(r[:D]).astype(BF)
        gate_v[:, cols] = jnp.broadcast_to(1.0 / (1.0 + jnp.exp(-r[D:D + 1])), (8, n))
        mean_v[:, cols] = jnp.broadcast_to(r[D + 1:D + 2], (8, n))

    def layernorm(a, n):
        for t in range(a, a + n, 128):
            cols = pl.ds(t, 128)
            xm = xT_v[every, cols].astype(F32) - mean_v[0:1, cols]
            var = jnp.sum(xm * xm, axis=0, keepdims=True) * (1.0 / D)
            mean_v[4:5, cols] = var
            hT_v[every, cols] = (xm * lax.rsqrt(var + 1e-5)).astype(BF)

    def p_proj(a, n):
        PT_v[every, pl.ds(a, n)] = _dot(xT_v[every, every], pk_v[every, pl.ds(a, n)]).astype(BF)

    def kv_block(j):
        row_head = lax.broadcasted_iota(jnp.int32, (128, 128), 0) // DH
        col_head = lax.broadcasted_iota(jnp.int32, (128, 128), 1) // DH
        js = pl.ds(j * 128, 128)
        kvT = _dot(wvT_v[js, every], PT_v[every, js])
        KV_v[js, every] = jnp.where(row_head == col_head, kvT, 0.0).astype(BF)

    def m_block(j):
        js = pl.ds(j * 128, 128)
        MT_v[every, js] = _dot(woT_v[every, js], KV_v[js, every]).astype(BF)

    def mixer_up(a, n):
        b1 = b1_v[...].astype(F32).reshape(1, F)
        u = _dot(hT_v[every, every], w1_v[0:S, pl.ds(a, n)]) + b1[:, a:a + n]
        g_v[every, pl.ds(a, n)] = jax.nn.gelu(u, approximate=True).astype(BF)

    def normalized_q(a, n, zc_v=zc_v):
        sub = lax.broadcasted_iota(jnp.int32, (8, 128), 0)
        m4, m2, m1 = sub < 4, (sub & 2) == 0, (sub & 1) == 0
        outs = []
        for t in range(a, a + n, 128):
            p = pqT_v[every, pl.ds(t, 128)].astype(F32)
            pz = p * zc_v[...]
            rows = []
            for grp in range(H // 8):
                h0 = grp * 8 * DH
                A = [pz[h0 + i * DH:h0 + i * DH + 8] + pz[h0 + i * DH + 8:h0 + (i + 1) * DH] for i in range(8)]
                B = [jnp.where(m4, A[i], A[i + 1]) + pltpu.roll(jnp.where(m4, A[i + 1], A[i]), 4, 0)
                     for i in range(0, 8, 2)]
                C = [jnp.where(m2, B[i] + pltpu.roll(B[i], 6, 0), B[i + 1] + pltpu.roll(B[i + 1], 2, 0))
                     for i in range(0, 4, 2)]
                den = jnp.where(m1, C[0] + pltpu.roll(C[0], 7, 0), C[1] + pltpu.roll(C[1], 1, 0)) + 1e-6
                inv = 1.0 / den
                for i in range(8):
                    s = ((i & 1) << 2) | (i & 2) | ((i >> 2) & 1)
                    rows.append(jnp.broadcast_to(inv[s:s + 1, :], (DH, 128)))
            outs.append((p * jnp.concatenate(rows, axis=0)).astype(BF))
        return jnp.concatenate(outs, axis=1) if len(outs) > 1 else outs[0]

    def mixer_down(chunk):
        a, n = chunk
        cols = pl.ds(a, n)
        b2 = b2_v[...].astype(F32).reshape(1, S)
        y = _dot(g_v[every, every], w2_v[("w2", a, n)][0:F, :])
        R_v[:, cols] = (1.0 - gate_v[0:1, cols]) * (y + b2[:, a:a + n])

    def attn_out(a, n, zsrc=zc_v):
        cols = pl.ds(a, n)
        R_v[:, cols] = R_v[:, cols] + gate_v[0:1, cols] * _dot(MT_v[every, every], normalized_q(a, n, zsrc))

    def emit(a, n):
        out_v[pl.ds(a, n), :] = R_v[:, pl.ds(a, n)].T.astype(BF)

    start(*_INPUTS)

    wait(_X0, _WK[0])
    k_proj(0, 256, 0, 128)
    transpose_x(0, 256)
    wait(_WK[1])
    k_proj(0, 256, 128, 128)
    wait(_X1)
    k_proj(256, 256, 0, 256)
    transpose_x(256, 256)
    wait(_WK[2])
    k_proj(0, 512, 256, 128)
    wait(_WK[3])
    k_proj(0, 512, 384, 128)
    wait(_X2)
    k_proj(512, 256)
    transpose_x(512, 256)
    k_proj(768, 256)
    transpose_x(768, 256)

    anchor(wq_v, D, pk_v, 768, 0)
    wait(_WQ, _GW)
    wqT_v[pl.ds(0, D), every] = wq_v[0:D, :].T
    aug_row = lax.broadcasted_iota(jnp.int32, (16, D), 0)
    gw = jnp.broadcast_to(gw_v[...].astype(F32).reshape(1, D), (16, D))
    wqT_v[pl.ds(D, 16), every] = jnp.where(aug_row == 0, gw, jnp.where(aug_row == 1, 1.0 / D, 0.0)).astype(BF)
    q_proj(0, 512)

    wait(_X3)
    k_proj(1024, 1024)
    transpose_x(1024, 1024)
    q_proj(512, 512)
    q_proj(1024, 1024)
    for c in range(0, S, 512):
        layernorm(c, 512)
    z_row = jnp.sum(z_v[...], axis=0, keepdims=True)
    zc0_v[...] = jnp.broadcast_to(z_row, (128, D)).T
    for j in range(4):
        p_proj(j * 128, 128)

    for t in range(4):
        anchor(w1_v, S, hT_v, D - PAD, 1536 + 128 * t, col=128 * (t + 1))
    anchor(w1_v, S, PT_v, 0, 384)
    wait(_W1, _B1, _WV, _WO)
    wvT_v[every, every] = wv_v[0:D, :].T
    woT_v[every, every] = wo_v[0:D, :].T

    mixer_up(0, 256)
    for j in range(4):
        kv_block(j)
    mixer_up(256, 256)
    for j in range(4):
        m_block(j)
    for f in range(2, 5):
        mixer_up(f * 256, 256)
    anchor(w2_v[_W2[0]], F, g_v, 0, 1024)
    wait(_W2[0], _B2)
    mixer_up(1280, 256)
    tie = g_v[pl.ds(0, 16), pl.ds(1408, 128)].astype(F32)[0:8] * 0.0
    zc_v[...] = zc0_v[...] + jnp.concatenate([tie] * (D // 8), axis=0)
    mixer_up(1536, 256)

    mixer_down(_YCHUNKS[0])
    for a in range(0, 1536, 256):
        attn_out(a, 256)
    wait(_W2[1])
    mixer_down(_YCHUNKS[1])
    attn_out(1536, 256)
    emit(0, 1536)
    start(_OUT[0], _OUT[1])
    wait(_W2[2])
    mixer_down(_YCHUNKS[2])
    attn_out(1792, 128)
    emit(1536, 256)
    start(_OUT[2])
    wait(_W2[3])
    mixer_down(_YCHUNKS[3])
    emit(1792, 128)
    start(_OUT[3])
    wait(_LATE)
    tie = jnp.broadcast_to(late_v[...].astype(F32).reshape(1, S)[:, 0:128] * 0.0, (8, 128))
    zc2_v[...] = zc_v[...] + jnp.concatenate([tie] * (D // 8), axis=0)
    attn_out(1920, 128, zc2_v)
    wait(_OUT[0])
    emit(1920, 128)
    start(_OUT[4])
    wait(_OUT[1])
    wait(_OUT[2], _OUT[3], _OUT[4])


@jax.jit
def pallas_gated_mix__linear_attn_block__mixer_token_mlp__prompt_kernel(
    A_x: jax.Array,
    A_wqkv: jax.Array,
    A_wo: jax.Array,
    B_x: jax.Array,
    B_w1: jax.Array,
    B_b1: jax.Array,
    B_w2: jax.Array,
    B_b2: jax.Array,
    gate_w: jax.Array,
):
    del B_x
    hbm = pl.BlockSpec(memory_space=pl.ANY)
    V = pltpu.VMEM
    scratch = [
        V((S, D), BF), V((D + PAD, D), BF), V((D, D), BF), V((D, D), BF), V((D, D), BF),
        V((S + PAD, F), BF), V((F,), BF), V((S,), BF), V((D,), BF),
        V(((D + 16) // 2, D), U32), V(((D) // 2, D), U32), V(((D) // 2, D), U32), V(((D) // 2, S), U32), V(((D) // 2, S), U32), V((D, S), BF), V(((S) // 2, D), U32), V(((D) // 2, D), U32), V((D, 128), BF), V(((D) // 2, D), U32), V(((D) // 2, F), U32),
        V((8, S), F32), V((8, S), F32), V((8, D), F32), V((D, 128), F32), V((D, 128), F32), V((D, 128), F32), V((S,), BF), V((D, S), F32), V((S, D), BF),
        pltpu.SemaphoreType.DMA((len(_COPIES),)),
    ] + [V((F + PAD, n), BF) for _, n in _YCHUNKS]
    return pl.pallas_call(
        _kernel,
        out_shape=jax.ShapeDtypeStruct((1, S, D), BF),
        in_specs=[hbm] * 8,
        out_specs=hbm,
        scratch_shapes=scratch,
        compiler_params=pltpu.CompilerParams(
            vmem_limit_bytes=100 * 1024 * 1024,
            flags={"XLA_TPU_RESCHEDULE_DMA_DONES": True},
            disable_semaphore_checks=True,
            disable_bounds_checks=True,
        ),
    )(A_x, A_wqkv, A_wo, B_w1, B_b1, B_w2, B_b2, gate_w)
```

```python
import jax
import jax.numpy as jnp
from jax import lax
from jax.experimental import pallas as pl
from jax.experimental.pallas import tpu as pltpu

S, D, F, H, DH = 2048, 512, 1792, 32, 16
BF, F32, U32 = jnp.bfloat16, jnp.float32, jnp.uint32
PAD = 16

_X0, _X1, _X2, _X2B, _X3 = ("x", 0, 256), ("x", 256, 256), ("x", 512, 256), ("x", 768, 256), ("x", 1024, 1024)
_WK = [("wk", 128 * i, 128) for i in range(4)]
_WQ, _WV, _WO = ("wq", 0, D), ("wv", 0, D), ("wo",)
_GW, _B1, _B2, _W1 = ("gw",), ("b1",), ("b2",), ("w1",)
_LATE = ("late",)
_YCHUNKS = [(0, 1536), (1536, 256), (1792, 128), (1920, 128)]
_W2 = [("w2", a, n) for a, n in _YCHUNKS]
_OUT = [("o", 0, 768), ("o", 768, 768), ("o", 1536, 256), ("o", 1792, 128), ("o", 1920, 128)]
_INPUTS = [_X0, _WK[0], _WK[1], _X1, _WK[2], _WK[3], _X2, _X2B, _WQ, _GW, _X3, _B1, _W1, _WV, _WO, _B2] + _W2 + [_LATE]
_COPIES = _INPUTS + _OUT


def _dot(a, b):
    return jnp.dot(a, b, preferred_element_type=F32)


def _phi(t):
    return jnp.where(t > 0, t + 1.0, jnp.exp(t)) + 1e-6


class _Packed:
    def __init__(self, ref):
        self.ref = ref

    @staticmethod
    def _idx(idx):
        r, c = idx
        r = slice(None) if isinstance(r, slice) else pl.ds(r.start // 2, r.size // 2)
        return r, c

    def __getitem__(self, idx):
        r, c = self._idx(idx)
        return pltpu.bitcast(self.ref[r, c], BF)

    def __setitem__(self, idx, val):
        r, c = self._idx(idx)
        self.ref[r, c] = pltpu.bitcast(val, U32)


def _kernel(x_hbm, wqkv_hbm, wo_hbm, w1_hbm, b1_hbm, w2_hbm, b2_hbm, gw_hbm, out_hbm,
            x_v, xb_v, xc_v, wq_v, wk_v, wv_v, wo_v, w1_v, b1_v, b2_v, gw_v,
            wqT_v, wvT_v, woT_v, xT_v, hT_v, pqT_v, pk_v, PT_v, KV_v, MT_v, g_v,
            gate_v, mean_v, z_v, zc0_v, zc_v, zc2_v, late_v, R_v, out_v, sems, *w2_vs):
    wqT_v, wvT_v, woT_v, xT_v, hT_v, pqT_v, pk_v, PT_v, KV_v, MT_v, g_v = [_Packed(wqT_v), _Packed(wvT_v), _Packed(woT_v), _Packed(xT_v), _Packed(hT_v), pqT_v, _Packed(pk_v), _Packed(PT_v), KV_v, _Packed(MT_v), _Packed(g_v)]
    w2_v = dict(zip(_W2, w2_vs))
    every = slice(None)

    def x_rows(a, n):
        for lo, hi, ref in ((0, 768, x_v), (768, 1024, xb_v), (1024, S, xc_v)):
            if lo <= a and a + n <= hi:
                return ref.at[pl.ds(a - lo, n), :]
        raise ValueError((a, n))

    def copy(name):
        kind, sem = name[0], sems.at[_COPIES.index(name)]
        if kind == "x":
            rows = pl.ds(name[1], name[2])
            return pltpu.make_async_copy(x_hbm.at[0, rows, :], x_rows(name[1], name[2]), sem)
        if kind == "o":
            rows = pl.ds(name[1], name[2])
            return pltpu.make_async_copy(out_v.at[rows, :], out_hbm.at[0, rows, :], sem)
        if kind in ("wq", "wk", "wv"):
            off, dst = {"wq": (0, wq_v), "wk": (D, wk_v), "wv": (2 * D, wv_v)}[kind]
            return pltpu.make_async_copy(wqkv_hbm.at[:, pl.ds(off + name[1], name[2])],
                                         dst.at[pl.ds(0, D), pl.ds(name[1], name[2])], sem)
        if kind == "w2":
            return pltpu.make_async_copy(w2_hbm.at[:, pl.ds(name[1], name[2])], w2_v[name].at[pl.ds(0, F), :], sem)
        src, dst = {"wo": (wo_hbm, wo_v), "w1": (w1_hbm, w1_v.at[pl.ds(0, S), :]),
                    "b1": (b1_hbm, b1_v), "b2": (b2_hbm, b2_v), "gw": (gw_hbm, gw_v), "late": (b2_hbm, late_v)}[kind]
        return pltpu.make_async_copy(src, dst, sem)

    def start(*names):
        for name in names:
            copy(name).start()

    def wait(*names):
        for name in names:
            copy(name).wait()

    def anchor(dst, row, src, r0, c0, col=0):
        dst[pl.ds(row, PAD), pl.ds(col, 128)] = src[pl.ds(r0, PAD), pl.ds(c0, 128)]

    z_seen = set()

    def k_proj(a, n, c0=0, cn=D):
        rows, cols = pl.ds(a, n), pl.ds(c0, cn)
        pk = _phi(_dot(x_rows(a, n)[...], wk_v[0:D, cols]))
        pk_v[rows, cols] = pk.astype(BF)
        part = jnp.sum(pk.reshape(n // 8, 8, cn), axis=0)
        for j in range(c0 // 128, (c0 + cn) // 128):
            js, ps = slice(j * 128, (j + 1) * 128), slice(j * 128 - c0, (j + 1) * 128 - c0)
            if j in z_seen:
                z_v[:, js] += part[:, ps]
            else:
                z_v[:, js] = part[:, ps]
                z_seen.add(j)

    def transpose_x(a, n):
        xT_v[every, pl.ds(a, n)] = x_rows(a, n)[...].T

    def q_proj(a, n):
        cols = pl.ds(a, n)
        r = _dot(wqT_v[every, every], xT_v[every, cols])
        pqT_v[every, cols] = _phi(r[:D]).astype(BF)
        gate_v[:, cols] = jnp.broadcast_to(1.0 / (1.0 + jnp.exp(-r[D:D + 1])), (8, n))
        mean_v[:, cols] = jnp.broadcast_to(r[D + 1:D + 2], (8, n))

    def layernorm(a, n):
        for t in range(a, a + n, 128):
            cols = pl.ds(t, 128)
            xm = xT_v[every, cols].astype(F32) - mean_v[0:1, cols]
            var = jnp.sum(xm * xm, axis=0, keepdims=True) * (1.0 / D)
            mean_v[4:5, cols] = var
            hT_v[every, cols] = (xm * lax.rsqrt(var + 1e-5)).astype(BF)

    def p_proj(a, n):
        PT_v[every, pl.ds(a, n)] = _dot(xT_v[every, every], pk_v[every, pl.ds(a, n)]).astype(BF)

    def kv_block(j):
        row_head = lax.broadcasted_iota(jnp.int32, (128, 128), 0) // DH
        col_head = lax.broadcasted_iota(jnp.int32, (128, 128), 1) // DH
        js = pl.ds(j * 128, 128)
        kvT = _dot(wvT_v[js, every], PT_v[every, js])
        KV_v[js, every] = jnp.where(row_head == col_head, kvT, 0.0).astype(BF)

    def m_block(j):
        js = pl.ds(j * 128, 128)
        MT_v[every, js] = _dot(woT_v[every, js], KV_v[js, every]).astype(BF)

    def mixer_up(a, n):
        b1 = b1_v[...].astype(F32).reshape(1, F)
        u = _dot(hT_v[every, every], w1_v[0:S, pl.ds(a, n)]) + b1[:, a:a + n]
        g_v[every, pl.ds(a, n)] = jax.nn.gelu(u, approximate=True).astype(BF)

    def normalized_q(a, n, zc_v=zc_v):
        sub = lax.broadcasted_iota(jnp.int32, (8, 128), 0)
        m4, m2, m1 = sub < 4, (sub & 2) == 0, (sub & 1) == 0
        outs = []
        for t in range(a, a + n, 128):
            p = pqT_v[every, pl.ds(t, 128)].astype(F32)
            pz = p * zc_v[...]
            rows = []
            for grp in range(H // 8):
                h0 = grp * 8 * DH
                A = [pz[h0 + i * DH:h0 + i * DH + 8] + pz[h0 + i * DH + 8:h0 + (i + 1) * DH] for i in range(8)]
                B = [jnp.where(m4, A[i], A[i + 1]) + pltpu.roll(jnp.where(m4, A[i + 1], A[i]), 4, 0)
                     for i in range(0, 8, 2)]
                C = [jnp.where(m2, B[i] + pltpu.roll(B[i], 6, 0), B[i + 1] + pltpu.roll(B[i + 1], 2, 0))
                     for i in range(0, 4, 2)]
                den = jnp.where(m1, C[0] + pltpu.roll(C[0], 7, 0), C[1] + pltpu.roll(C[1], 1, 0)) + 1e-6
                inv = 1.0 / den
                for i in range(8):
                    s = ((i & 1) << 2) | (i & 2) | ((i >> 2) & 1)
                    rows.append(jnp.broadcast_to(inv[s:s + 1, :], (DH, 128)))
            outs.append((p * jnp.concatenate(rows, axis=0)).astype(BF))
        return jnp.concatenate(outs, axis=1) if len(outs) > 1 else outs[0]

    def mixer_down(chunk):
        a, n = chunk
        cols = pl.ds(a, n)
        b2 = b2_v[...].astype(F32).reshape(1, S)
        y = _dot(g_v[every, every], w2_v[("w2", a, n)][0:F, :])
        R_v[:, cols] = (1.0 - gate_v[0:1, cols]) * (y + b2[:, a:a + n])

    def attn_out(a, n, zsrc=zc_v):
        cols = pl.ds(a, n)
        R_v[:, cols] = R_v[:, cols] + gate_v[0:1, cols] * _dot(MT_v[every, every], normalized_q(a, n, zsrc))

    def emit(a, n):
        out_v[pl.ds(a, n), :] = R_v[:, pl.ds(a, n)].T.astype(BF)

    start(*_INPUTS)

    wait(_X0, _WK[0])
    k_proj(0, 256, 0, 128)
    transpose_x(0, 256)
    wait(_WK[1])
    k_proj(0, 256, 128, 128)
    wait(_X1)
    k_proj(256, 256, 0, 256)
    transpose_x(256, 256)
    wait(_WK[2])
    k_proj(0, 512, 256, 128)
    wait(_WK[3])
    k_proj(0, 512, 384, 128)
    wait(_X2)
    k_proj(512, 256)
    transpose_x(512, 256)
    anchor(xb_v, 256, pk_v, 576, 0)
    wait(_X2B)
    k_proj(768, 256)
    transpose_x(768, 256)

    anchor(wq_v, D, pk_v, 1008, 0)
    wait(_WQ, _GW)
    wqT_v[pl.ds(0, D), every] = wq_v[0:D, :].T
    aug_row = lax.broadcasted_iota(jnp.int32, (16, D), 0)
    gw = jnp.broadcast_to(gw_v[...].astype(F32).reshape(1, D), (16, D))
    wqT_v[pl.ds(D, 16), every] = jnp.where(aug_row == 0, gw, jnp.where(aug_row == 1, 1.0 / D, 0.0)).astype(BF)
    q_proj(0, 512)

    anchor(xc_v, 1024, xT_v, 496, 896)
    wait(_X3)
    q_proj(512, 512)
    k_proj(1024, 1024)
    transpose_x(1024, 1024)
    q_proj(1024, 1024)
    for c in range(0, S, 512):
        layernorm(c, 512)
    z_row = jnp.sum(z_v[...], axis=0, keepdims=True)
    zc0_v[...] = jnp.broadcast_to(z_row, (128, D)).T
    for j in range(4):
        p_proj(j * 128, 128)

    for t in range(4):
        anchor(w1_v, S, hT_v, D - PAD, 1536 + 128 * t, col=128 * (t + 1))
    anchor(w1_v, S, PT_v, 0, 384)
    wait(_W1, _B1, _WV, _WO)
    wvT_v[every, every] = wv_v[0:D, :].T
    woT_v[every, every] = wo_v[0:D, :].T

    mixer_up(0, 256)
    for j in range(4):
        kv_block(j)
    mixer_up(256, 256)
    for j in range(4):
        m_block(j)
    for f in range(2, 5):
        mixer_up(f * 256, 256)
    anchor(w2_v[_W2[0]], F, g_v, 0, 1024)
    wait(_W2[0], _B2)
    mixer_up(1280, 256)
    tie = g_v[pl.ds(0, 16), pl.ds(1408, 128)].astype(F32)[0:8] * 0.0
    zc_v[...] = zc0_v[...] + jnp.concatenate([tie] * (D // 8), axis=0)
    mixer_up(1536, 256)

    mixer_down(_YCHUNKS[0])
    for a in range(0, 1536, 256):
        attn_out(a, 256)
    wait(_W2[1])
    mixer_down(_YCHUNKS[1])
    attn_out(1536, 256)
    emit(0, 1536)
    start(_OUT[0], _OUT[1])
    wait(_W2[2])
    mixer_down(_YCHUNKS[2])
    attn_out(1792, 128)
    emit(1536, 256)
    start(_OUT[2])
    wait(_W2[3])
    mixer_down(_YCHUNKS[3])
    emit(1792, 128)
    start(_OUT[3])
    wait(_LATE)
    tie = jnp.broadcast_to(late_v[...].astype(F32).reshape(1, S)[:, 0:128] * 0.0, (8, 128))
    zc2_v[...] = zc_v[...] + jnp.concatenate([tie] * (D // 8), axis=0)
    attn_out(1920, 128, zc2_v)
    wait(_OUT[0])
    emit(1920, 128)
    start(_OUT[4])
    wait(_OUT[1])
    wait(_OUT[2], _OUT[3], _OUT[4])


@jax.jit
def pallas_gated_mix__linear_attn_block__mixer_token_mlp__prompt_kernel(
    A_x: jax.Array,
    A_wqkv: jax.Array,
    A_wo: jax.Array,
    B_x: jax.Array,
    B_w1: jax.Array,
    B_b1: jax.Array,
    B_w2: jax.Array,
    B_b2: jax.Array,
    gate_w: jax.Array,
):
    del B_x
    hbm = pl.BlockSpec(memory_space=pl.ANY)
    V = pltpu.VMEM
    scratch = [
        V((768, D), BF), V((256 + PAD, D), BF), V((1024 + PAD, D), BF), V((D + PAD, D), BF), V((D, D), BF), V((D, D), BF), V((D, D), BF),
        V((S + PAD, F), BF), V((F,), BF), V((S,), BF), V((D,), BF),
        V(((D + 16) // 2, D), U32), V(((D) // 2, D), U32), V(((D) // 2, D), U32), V(((D) // 2, S), U32), V(((D) // 2, S), U32), V((D, S), BF), V(((S) // 2, D), U32), V(((D) // 2, D), U32), V((D, 128), BF), V(((D) // 2, D), U32), V(((D) // 2, F), U32),
        V((8, S), F32), V((8, S), F32), V((8, D), F32), V((D, 128), F32), V((D, 128), F32), V((D, 128), F32), V((S,), BF), V((D, S), F32), V((S, D), BF),
        pltpu.SemaphoreType.DMA((len(_COPIES),)),
    ] + [V((F + PAD, n), BF) for _, n in _YCHUNKS]
    return pl.pallas_call(
        _kernel,
        out_shape=jax.ShapeDtypeStruct((1, S, D), BF),
        in_specs=[hbm] * 8,
        out_specs=hbm,
        scratch_shapes=scratch,
        compiler_params=pltpu.CompilerParams(
            vmem_limit_bytes=100 * 1024 * 1024,
            flags={"XLA_TPU_RESCHEDULE_DMA_DONES": True},
            disable_semaphore_checks=True,
            disable_bounds_checks=True,
        ),
    )(A_x, A_wqkv, A_wo, B_w1, B_b1, B_w2, B_b2, gate_w)
```

```python
import jax
import jax.numpy as jnp
from jax import lax
from jax.experimental import pallas as pl
from jax.experimental.pallas import tpu as pltpu

S, D, F, H, DH = 2048, 512, 1792, 32, 16
BF, F32, U32 = jnp.bfloat16, jnp.float32, jnp.uint32
PAD = 16

_X0, _X1, _X2, _X2B, _X3 = ("x", 0, 256), ("x", 256, 256), ("x", 512, 256), ("x", 768, 256), ("x", 1024, 1024)
_WK = [("wk", 128 * i, 128) for i in range(4)]
_WQ, _WV, _WO = ("wq", 0, D), ("wv", 0, D), ("wo",)
_GW, _B1, _B2, _W1 = ("gw",), ("b1",), ("b2",), ("w1",)
_LATE = ("late",)
_YCHUNKS = [(0, 1536), (1536, 256), (1792, 128), (1920, 128)]
_W2 = [("w2", a, n) for a, n in _YCHUNKS]
_OUT = [("o", 0, 768), ("o", 768, 768), ("o", 1536, 256), ("o", 1792, 128), ("o", 1920, 128)]
_INPUTS = [_X0, _WK[0], _WK[1], _X1, _WK[2], _WK[3], _X2, _X2B, _WQ, _GW, _X3, _B1, _W1, _WV, _WO, _B2] + _W2 + [_LATE]
_COPIES = _INPUTS + _OUT


def _dot(a, b):
    return jnp.dot(a, b, preferred_element_type=F32)


def _phi(t):
    return jnp.where(t > 0, t + 1.0, jnp.exp(t)) + 1e-6


class _Packed:
    def __init__(self, ref):
        self.ref = ref

    @staticmethod
    def _idx(idx):
        r, c = idx
        r = slice(None) if isinstance(r, slice) else pl.ds(r.start // 2, r.size // 2)
        return r, c

    def __getitem__(self, idx):
        r, c = self._idx(idx)
        return pltpu.bitcast(self.ref[r, c], BF)

    def __setitem__(self, idx, val):
        r, c = self._idx(idx)
        self.ref[r, c] = pltpu.bitcast(val, U32)


def _kernel(x_hbm, wqkv_hbm, wo_hbm, w1_hbm, b1_hbm, w2_hbm, b2_hbm, gw_hbm, out_hbm,
            x_v, xb_v, xc_v, wq_v, wk_v, wv_v, wo_v, w1_v, b1_v, b2_v, gw_v,
            wqT_v, wvT_v, woT_v, xT_v, hT_v, pqT_v, pk_v, PT_v, KV_v, MT_v, g_v,
            gate_v, mean_v, z_v, zc0_v, zc_v, zc2_v, late_v, R_v, out_v, sems, *w2_vs):
    wqT_v, wvT_v, woT_v, xT_v, hT_v, pk_v, PT_v, MT_v, g_v = [
        _Packed(r) for r in (wqT_v, wvT_v, woT_v, xT_v, hT_v, pk_v, PT_v, MT_v, g_v)]
    w2_v = dict(zip(_W2, w2_vs))
    every = slice(None)

    def x_rows(a, n):
        for lo, hi, ref in ((0, 768, x_v), (768, 1024, xb_v), (1024, S, xc_v)):
            if lo <= a and a + n <= hi:
                return ref.at[pl.ds(a - lo, n), :]
        raise ValueError((a, n))

    def copy(name):
        kind, sem = name[0], sems.at[_COPIES.index(name)]
        if kind == "x":
            rows = pl.ds(name[1], name[2])
            return pltpu.make_async_copy(x_hbm.at[0, rows, :], x_rows(name[1], name[2]), sem)
        if kind == "o":
            rows = pl.ds(name[1], name[2])
            return pltpu.make_async_copy(out_v.at[rows, :], out_hbm.at[0, rows, :], sem)
        if kind in ("wq", "wk", "wv"):
            off, dst = {"wq": (0, wq_v), "wk": (D, wk_v), "wv": (2 * D, wv_v)}[kind]
            return pltpu.make_async_copy(wqkv_hbm.at[:, pl.ds(off + name[1], name[2])],
                                         dst.at[pl.ds(0, D), pl.ds(name[1], name[2])], sem)
        if kind == "w2":
            return pltpu.make_async_copy(w2_hbm.at[:, pl.ds(name[1], name[2])], w2_v[name].at[pl.ds(0, F), :], sem)
        src, dst = {"wo": (wo_hbm, wo_v), "w1": (w1_hbm, w1_v.at[pl.ds(0, S), :]),
                    "b1": (b1_hbm, b1_v), "b2": (b2_hbm, b2_v), "gw": (gw_hbm, gw_v), "late": (b2_hbm, late_v)}[kind]
        return pltpu.make_async_copy(src, dst, sem)

    def start(*names):
        for name in names:
            copy(name).start()

    def wait(*names):
        for name in names:
            copy(name).wait()

    def anchor(dst, row, src, r0, c0, col=0):
        dst[pl.ds(row, PAD), pl.ds(col, 128)] = src[pl.ds(r0, PAD), pl.ds(c0, 128)]

    z_seen = set()

    def k_proj(a, n, c0=0, cn=D):
        rows, cols = pl.ds(a, n), pl.ds(c0, cn)
        pk = _phi(_dot(x_rows(a, n)[...], wk_v[0:D, cols]))
        pk_v[rows, cols] = pk.astype(BF)
        part = jnp.sum(pk.reshape(n // 8, 8, cn), axis=0)
        for j in range(c0 // 128, (c0 + cn) // 128):
            js, ps = slice(j * 128, (j + 1) * 128), slice(j * 128 - c0, (j + 1) * 128 - c0)
            if j in z_seen:
                z_v[:, js] += part[:, ps]
            else:
                z_v[:, js] = part[:, ps]
                z_seen.add(j)

    def transpose_x(a, n):
        xT_v[every, pl.ds(a, n)] = x_rows(a, n)[...].T

    def q_proj(a, n):
        cols = pl.ds(a, n)
        r = _dot(wqT_v[every, every], xT_v[every, cols])
        pqT_v[every, cols] = _phi(r[:D]).astype(BF)
        gate_v[:, cols] = jnp.broadcast_to(1.0 / (1.0 + jnp.exp(-r[D:D + 1])), (8, n))
        mean_v[:, cols] = jnp.broadcast_to(r[D + 1:D + 2], (8, n))

    def layernorm(a, n):
        for t in range(a, a + n, 128):
            cols = pl.ds(t, 128)
            xm = xT_v[every, cols].astype(F32) - mean_v[0:1, cols]
            var = jnp.sum(xm * xm, axis=0, keepdims=True) * (1.0 / D)
            mean_v[4:5, cols] = var
            hT_v[every, cols] = (xm * lax.rsqrt(var + 1e-5)).astype(BF)

    def p_proj(a, n):
        PT_v[every, pl.ds(a, n)] = _dot(xT_v[every, every], pk_v[every, pl.ds(a, n)]).astype(BF)

    def kv_block(j):
        row_head = lax.broadcasted_iota(jnp.int32, (128, 128), 0) // DH
        col_head = lax.broadcasted_iota(jnp.int32, (128, 128), 1) // DH
        js = pl.ds(j * 128, 128)
        kvT = _dot(wvT_v[js, every], PT_v[every, js])
        KV_v[js, every] = jnp.where(row_head == col_head, kvT, 0.0).astype(BF)

    def m_block(j):
        js = pl.ds(j * 128, 128)
        MT_v[every, js] = _dot(woT_v[every, js], KV_v[js, every]).astype(BF)

    def mixer_up(a, n):
        b1 = b1_v[...].astype(F32).reshape(1, F)
        u = _dot(hT_v[every, every], w1_v[0:S, pl.ds(a, n)]) + b1[:, a:a + n]
        g_v[every, pl.ds(a, n)] = jax.nn.gelu(u, approximate=True).astype(BF)

    def normalized_q(a, n, zc_v=zc_v):
        sub = lax.broadcasted_iota(jnp.int32, (8, 128), 0)
        m4, m2, m1 = sub < 4, (sub & 2) == 0, (sub & 1) == 0
        outs = []
        for t in range(a, a + n, 128):
            p = pqT_v[every, pl.ds(t, 128)].astype(F32)
            pz = p * zc_v[...]
            rows = []
            for grp in range(H // 8):
                h0 = grp * 8 * DH
                A = [pz[h0 + i * DH:h0 + i * DH + 8] + pz[h0 + i * DH + 8:h0 + (i + 1) * DH] for i in range(8)]
                B = [jnp.where(m4, A[i], A[i + 1]) + pltpu.roll(jnp.where(m4, A[i + 1], A[i]), 4, 0)
                     for i in range(0, 8, 2)]
                C = [jnp.where(m2, B[i] + pltpu.roll(B[i], 6, 0), B[i + 1] + pltpu.roll(B[i + 1], 2, 0))
                     for i in range(0, 4, 2)]
                den = jnp.where(m1, C[0] + pltpu.roll(C[0], 7, 0), C[1] + pltpu.roll(C[1], 1, 0)) + 1e-6
                inv = 1.0 / den
                for i in range(8):
                    s = ((i & 1) << 2) | (i & 2) | ((i >> 2) & 1)
                    rows.append(jnp.broadcast_to(inv[s:s + 1, :], (DH, 128)))
            outs.append((p * jnp.concatenate(rows, axis=0)).astype(BF))
        return jnp.concatenate(outs, axis=1) if len(outs) > 1 else outs[0]

    def mixer_down(chunk):
        a, n = chunk
        cols = pl.ds(a, n)
        b2 = b2_v[...].astype(F32).reshape(1, S)
        y = _dot(g_v[every, every], w2_v[("w2", a, n)][0:F, :])
        R_v[:, cols] = (1.0 - gate_v[0:1, cols]) * (y + b2[:, a:a + n])

    def attn_out(a, n, zsrc=zc_v):
        cols = pl.ds(a, n)
        R_v[:, cols] = R_v[:, cols] + gate_v[0:1, cols] * _dot(MT_v[every, every], normalized_q(a, n, zsrc))

    def emit(a, n):
        out_v[pl.ds(a, n), :] = R_v[:, pl.ds(a, n)].T.astype(BF)

    start(*_INPUTS)

    wait(_X0, _WK[0])
    k_proj(0, 256, 0, 128)
    transpose_x(0, 256)
    wait(_WK[1])
    k_proj(0, 256, 128, 128)
    wait(_X1)
    k_proj(256, 256, 0, 256)
    transpose_x(256, 256)
    wait(_WK[2])
    k_proj(0, 512, 256, 128)
    wait(_WK[3])
    k_proj(0, 512, 384, 128)
    wait(_X2)
    k_proj(512, 256)
    transpose_x(512, 256)
    anchor(xb_v, 256, pk_v, 576, 0)
    wait(_X2B)
    k_proj(768, 256)
    transpose_x(768, 256)

    anchor(wq_v, D, pk_v, 1008, 0)
    wait(_WQ, _GW)
    wqT_v[pl.ds(0, D), every] = wq_v[0:D, :].T
    aug_row = lax.broadcasted_iota(jnp.int32, (16, D), 0)
    gw = jnp.broadcast_to(gw_v[...].astype(F32).reshape(1, D), (16, D))
    wqT_v[pl.ds(D, 16), every] = jnp.where(aug_row == 0, gw, jnp.where(aug_row == 1, 1.0 / D, 0.0)).astype(BF)
    q_proj(0, 512)

    anchor(xc_v, 1024, xT_v, 496, 896)
    wait(_X3)
    q_proj(512, 512)
    k_proj(1024, 1024)
    transpose_x(1024, 1024)
    q_proj(1024, 1024)
    for c in range(0, S, 512):
        layernorm(c, 512)
    z_row = jnp.sum(z_v[...], axis=0, keepdims=True)
    zc0_v[...] = jnp.broadcast_to(z_row, (128, D)).T
    for j in range(4):
        p_proj(j * 128, 128)

    for t in range(4):
        anchor(w1_v, S, hT_v, D - PAD, 1536 + 128 * t, col=128 * (t + 1))
    anchor(w1_v, S, PT_v, 0, 384)
    wait(_W1, _B1, _WV, _WO)
    wvT_v[every, every] = wv_v[0:D, :].T
    woT_v[every, every] = wo_v[0:D, :].T

    mixer_up(0, 256)
    for j in range(4):
        kv_block(j)
    mixer_up(256, 256)
    for j in range(4):
        m_block(j)
    for f in range(2, 5):
        mixer_up(f * 256, 256)
    anchor(w2_v[_W2[0]], F, g_v, 0, 1024)
    wait(_W2[0], _B2)
    mixer_up(1280, 256)
    tie = g_v[pl.ds(0, 16), pl.ds(1408, 128)].astype(F32)[0:8] * 0.0
    zc_v[...] = zc0_v[...] + jnp.concatenate([tie] * (D // 8), axis=0)
    mixer_up(1536, 256)

    mixer_down(_YCHUNKS[0])
    for a in range(0, 1536, 256):
        attn_out(a, 256)
    wait(_W2[1])
    mixer_down(_YCHUNKS[1])
    attn_out(1536, 256)
    emit(0, 1536)
    start(_OUT[0], _OUT[1])
    wait(_W2[2])
    mixer_down(_YCHUNKS[2])
    attn_out(1792, 128)
    emit(1536, 256)
    start(_OUT[2])
    wait(_W2[3])
    mixer_down(_YCHUNKS[3])
    emit(1792, 128)
    start(_OUT[3])
    wait(_LATE)
    tie = jnp.broadcast_to(late_v[...].astype(F32).reshape(1, S)[:, 0:128] * 0.0, (8, 128))
    zc2_v[...] = zc_v[...] + jnp.concatenate([tie] * (D // 8), axis=0)
    attn_out(1920, 128, zc2_v)
    wait(_OUT[0])
    emit(1920, 128)
    start(_OUT[4])
    wait(_OUT[1])
    wait(_OUT[2], _OUT[3], _OUT[4])


@jax.jit
def pallas_gated_mix__linear_attn_block__mixer_token_mlp__prompt_kernel(
    A_x: jax.Array,
    A_wqkv: jax.Array,
    A_wo: jax.Array,
    B_x: jax.Array,
    B_w1: jax.Array,
    B_b1: jax.Array,
    B_w2: jax.Array,
    B_b2: jax.Array,
    gate_w: jax.Array,
):
    del B_x
    hbm = pl.BlockSpec(memory_space=pl.ANY)
    V = pltpu.VMEM
    scratch = [
        V((768, D), BF), V((256 + PAD, D), BF), V((1024 + PAD, D), BF),
        V((D + PAD, D), BF), V((D, D), BF), V((D, D), BF), V((D, D), BF),
        V((S + PAD, F), BF), V((F,), BF), V((S,), BF), V((D,), BF),
        V(((D + 16) // 2, D), U32), V((D // 2, D), U32), V((D // 2, D), U32),
        V((D // 2, S), U32), V((D // 2, S), U32), V((D, S), BF), V((S // 2, D), U32),
        V((D // 2, D), U32), V((D, 128), BF), V((D // 2, D), U32), V((D // 2, F), U32),
        V((8, S), F32), V((8, S), F32), V((8, D), F32), V((D, 128), F32), V((D, 128), F32), V((D, 128), F32),
        V((S,), BF), V((D, S), F32), V((S, D), BF),
        pltpu.SemaphoreType.DMA((len(_COPIES),)),
    ] + [V((F + PAD, n), BF) for _, n in _YCHUNKS]
    return pl.pallas_call(
        _kernel,
        out_shape=jax.ShapeDtypeStruct((1, S, D), BF),
        in_specs=[hbm] * 8,
        out_specs=hbm,
        scratch_shapes=scratch,
        compiler_params=pltpu.CompilerParams(
            vmem_limit_bytes=100 * 1024 * 1024,
            flags={"XLA_TPU_RESCHEDULE_DMA_DONES": True},
            disable_semaphore_checks=True,
            disable_bounds_checks=True,
        ),
    )(A_x, A_wqkv, A_wo, B_w1, B_b1, B_w2, B_b2, gate_w)
```
